```python
import os as _os
_os.environ.setdefault("JAX_PLATFORMS", "cpu")
import jax
import jax.numpy as jnp

def _softmax(x, axis=-1):
    return jax.nn.softmax(x, axis=axis)
def _gelu(x):
    return jax.nn.gelu(x, approximate=True)
def _silu(x):
    return jax.nn.silu(x)
def _sigmoid(x):
    return jax.nn.sigmoid(x)
def _layernorm(x, axis=-1, eps=1e-5):
    m = jnp.mean(x, axis=axis, keepdims=True)
    v = jnp.var(x, axis=axis, keepdims=True)
    return (x - m) / jnp.sqrt(v + eps)
def _scatter_add(tgt, idx, src, axis=0):
    return tgt.at[idx].add(src)
def _segment_sum(src, seg, n):
    return jax.ops.segment_sum(src, seg, n)
class _Rng:
    def __init__(self, key):
        self._k = key
    def _next(self):
        self._k, sub = jax.random.split(self._k)
        return sub
    def normal(self, shape):
        return jax.random.normal(self._next(), shape, dtype=jnp.bfloat16)
    def randint(self, lo, hi, shape):
        return jax.random.randint(self._next(), shape, lo, hi, dtype=jnp.int32)
    def uniform(self, shape, lo=0.0, hi=1.0):
        return jax.random.uniform(self._next(), shape, jnp.bfloat16, lo, hi)
    def permutation(self, n):
        return jax.random.permutation(self._next(), n)


kernel_name = 'sequential_preLN__mha_block__mixer_token_mlp__prompt'

def setup_inputs():
    _rng = _Rng(jax.random.key(int.from_bytes(__import__("os").urandom(4), "little")))
    _w = (lambda a: (lambda t: t.astype(jnp.bfloat16) if jnp.issubdtype(t.dtype, jnp.floating) else t)(jnp.asarray(a)))
    def _A_setup():
        B, S, D, H = 1, 2048, 448, 16
        return {
            "x": _w((lambda *s: _rng.normal(s) * 0.05)(B, S, D)),
            "wqkv": _w((lambda *s: _rng.normal(s) * 0.05)(D, 3 * D)),
            "wo": _w((lambda *s: _rng.normal(s) * 0.05)(D, D)),
        }
    _A_in = _A_setup()

    def _B_setup():
        B, S, D, F = 1, 2048, 448, 1792
        return {
            "x": _w((lambda *s: _rng.normal(s) * 0.05)(B, S, D)),
            "w1": _w((lambda *s: _rng.normal(s) * 0.2)(S, F) * (S ** -0.5)),
            "b1": _w((lambda *s: _rng.normal(s) * 0.2)(F) * 0.02),
            "w2": _w((lambda *s: _rng.normal(s) * 0.2)(F, S) * (F ** -0.5)),
            "b2": _w((lambda *s: _rng.normal(s) * 0.05)(S) * 0.02),
        }
    _B_in = _B_setup()

    return {
        "A_x": _A_in["x"],
        "A_wqkv": _A_in["wqkv"],
        "A_wo": _A_in["wo"],
        "B_x": _B_in["x"],
        "B_w1": _B_in["w1"],
        "B_b1": _B_in["b1"],
        "B_w2": _B_in["w2"],
        "B_b2": _B_in["b2"],
    }

def reference(A_x, A_wqkv, A_wo, B_x, B_w1, B_b1, B_w2, B_b2):
    def _A_ref(x, wqkv, wo):
        B, S, D = x.shape
        H = 16
        Dh = D // H
        qkv = (lambda x, *d: x.transpose(*d))((x @ wqkv).reshape(B, S, 3, H, Dh), 2, 0, 3, 1, 4)
        q, k, v = qkv[0], qkv[1], qkv[2]
        scores = jnp.einsum("bhqd,bhkd->bhqk", q, k) * (Dh ** -0.5)
        p = _softmax(scores, axis=-1)
        o = jnp.einsum("bhqk,bhkd->bhqd", p, v)
        return (lambda x, *d: x.transpose(*d))(o, 0, 2, 1, 3).reshape(B, S, D) @ wo

    def _B_ref(x, w1, b1, w2, b2):
        B, S, D = x.shape
        h = _layernorm(x, axis=-1)
        u = jnp.einsum("bsd,sf->bdf", h, w1) + b1
        u = _gelu(u)
        y = jnp.einsum("bdf,fs->bds", u, w2) + b2
        return (lambda x, *d: x.transpose(*d))(y, 0, 2, 1)

    x = A_x
    h = x + _A_ref(_layernorm(x, axis=-1), A_wqkv, A_wo)
    h2 = h + _B_ref(_layernorm(h, axis=-1), B_w1, B_b1, B_w2, B_b2)
    return h2
```

```python
import functools
import math

import jax
import jax.numpy as jnp
import jax.experimental.pallas as pl
import jax.experimental.pallas.tpu as pltpu

_H = 16
_HP = 32
_G = 4
_BQ = 512
_KC = 256
_UN = 8
_SC = 512
_FC = 128
_EC = 256
_ORDER_UP = (5, 3, 2, 4, 6, 1, 7)
_ORDER_DOWN = (2, 5, 3, 4, 1, 7, 6)
_EPS = 1e-5
_SUM_LO, _SUM_HI = 2.0 ** -10, 2.0 ** 70
_NUM_LO, _NUM_HI = 2.0 ** -85, 2.0 ** 120

_BF = jnp.bfloat16
_F32 = jnp.float32


def _dot(a, b):
    return jnp.dot(a, b, preferred_element_type=_F32)


def _chunk(c, size):
    if isinstance(c, int):
        return pl.ds(c * size, size)
    return pl.ds(pl.multiple_of(c * size, size), size)


def _store_lhs(ref, cols, a11, a12, a21, a22):
    for n, a in enumerate((a11 + a22, a21 + a22, a11, a22, a11 + a12, a21 - a11, a12 - a22)):
        ref[n, :, cols] = a.astype(_BF)


def _strassen(a_ref, b_ref, left, right, order):
    kh = b_ref.shape[0] // 2
    blocks = {11: (slice(0, kh), left), 12: (slice(0, kh), right),
              21: (slice(kh, 2 * kh), left), 22: (slice(kh, 2 * kh), right)}

    def b(i, j=None, sign=1):
        if j is None:
            return b_ref[blocks[i]]
        x, y = b_ref[blocks[i]].astype(_F32), b_ref[blocks[j]].astype(_F32)
        return (x + y if sign > 0 else x - y).astype(_BF)

    products = {
        1: ((11, 22), ((0, 1), (3, 1))),
        2: ((11,), ((2, 1), (3, -1))),
        3: ((12, 22, -1), ((1, 1), (3, 1))),
        4: ((21, 11, -1), ((0, 1), (2, 1))),
        5: ((22,), ((0, -1), (1, 1))),
        6: ((11, 12), ((3, 1),)),
        7: ((21, 22), ((0, 1),)),
    }
    out = [None] * 4
    for n in order:
        factor, targets = products[n]
        m = _dot(a_ref[n - 1], b(*factor))
        for t, sign in targets:
            if out[t] is None:
                out[t] = m if sign > 0 else -m
            else:
                out[t] = out[t] + m if sign > 0 else out[t] - m
    return out


def _ln_t(xt):
    n = xt.shape[0]
    m = jnp.sum(xt, axis=0, keepdims=True) * (1.0 / n)
    c = xt - m
    v = jnp.sum(c * c, axis=0, keepdims=True) * (1.0 / n)
    return c * jax.lax.rsqrt(v + _EPS)


def _gelu(x):
    c = math.sqrt(2.0 / math.pi)
    inner = x * (c + (c * 0.044715) * (x * x))
    hx = 0.5 * x
    return hx + hx * jnp.tanh(inner)


def _kernel(x_hbm, wqkv_hbm, wo_hbm, b1_in, b2_in, w1_hbm, w2_hbm, out_hbm,
            x_ref, wv_ref, wqk_ref, wo_ref, w1_ref, w2_ref, b1_ref, b2_ref,
            ht_ref, qt_ref, k_ref, vt_ref, ot_ref, p0_ref, p1_ref, hn_ref, g_ref,
            ob_ref, wot_ref, in_sem, o_sem):
    D, S = x_ref.shape
    F = w1_ref.shape[1]
    Dh = D // _H
    Dm = D // 2
    GW = _G * Dh
    nq = S // _BQ
    n_steps = _H * nq

    first, rest = pl.ds(0, _SC), pl.ds(_SC, S - _SC)
    qk_cols, v_cols = pl.ds(0, 2 * D), pl.ds(2 * D, D)
    loads = [pltpu.make_async_copy(src, dst, in_sem.at[n]) for n, (src, dst) in enumerate([
        (x_hbm.at[:, first], x_ref.at[:, first]),
        (wqkv_hbm.at[:, v_cols], wv_ref),
        (wqkv_hbm.at[:, qk_cols], wqk_ref),
        (x_hbm.at[:, rest], x_ref.at[:, rest]),
        (wo_hbm, wo_ref), (w1_hbm, w1_ref), (w2_hbm, w2_ref)])]
    x0_cp, wv_cp, wqk_cp, x1_cp, wo_cp, w1_cp, w2_cp = loads
    x0_cp.start()
    wv_cp.start()

    q_scale = (Dh ** -0.5) * math.log2(math.e)
    row = jax.lax.broadcasted_iota(jnp.int32, (_HP - Dh, _SC), 0)
    ones_row = jnp.where(row == 0, 1.0, 0.0).astype(_F32)

    p1_ref[...] = jnp.zeros(p1_ref.shape, _BF)
    b1_ref[...] = b1_in[...].astype(_F32).reshape(1, F)
    b2_ref[...] = b2_in[...].astype(_F32).reshape(1, S)

    x0_cp.wait()
    wv_cp.wait()
    wqk_cp.start()
    wvt = wv_ref[...].astype(_F32).T.astype(_BF)
    for c in range(S // _SC):
        sl = _chunk(c, _SC)
        if c == 1:
            x1_cp.wait()
            for cp in (wo_cp, w1_cp, w2_cp):
                cp.start()
        ht = _ln_t(x_ref[:, sl].astype(_F32)).astype(_BF)
        vt = _dot(wvt, ht)
        for h in range(_H):
            vh = jnp.concatenate([vt[h * Dh:(h + 1) * Dh], ones_row], axis=0)
            vt_ref[h, :, sl] = vh.astype(_BF)
        if c == 0:
            wqk_cp.wait()
            x1_cp.start()
            wqkt = wqk_ref[...].astype(_F32).T.astype(_BF)
        kt = _dot(wqkt[D:], ht)
        zpad = jnp.zeros((128 - GW, _SC), _F32)
        for g in range(_H // _G):
            kg = jnp.concatenate([kt[g * GW:(g + 1) * GW], zpad], axis=0)
            k_ref[g, sl, :] = kg.T.astype(_BF)
        qt_ref[:, sl] = _dot(wqkt[:D], ht) * q_scale

    grow = jax.lax.broadcasted_iota(jnp.int32, (GW, _BQ), 0)

    def q_weights(i):
        h = i // nq
        g = h // _G
        lo = (h % _G) * Dh
        qs = pl.ds(pl.multiple_of((i % nq) * _BQ, _BQ), _BQ)
        q = qt_ref[pl.ds(pl.multiple_of(g * GW, 8), GW), qs]
        q = jnp.where((grow >= lo) & (grow < lo + Dh), q, 0.0)
        q = jnp.concatenate([q, jnp.zeros((128 - GW, _BQ), _F32)], axis=0)
        return g, q.astype(_BF)

    def q_slice(i):
        return pl.ds(pl.multiple_of((i % nq) * _BQ, _BQ), _BQ)

    def store_o(i, acc):
        hs = pl.ds(pl.multiple_of((i // nq) * _HP, _HP), _HP)
        den = jnp.maximum(acc[Dh:Dh + 1, :], _SUM_LO)
        ot_ref[hs, q_slice(i)] = (acc * (1.0 / den)).astype(_BF)

    def in_range(acc):
        mag = jnp.abs(acc)
        den = acc[Dh:Dh + 1, :]
        finite = jnp.min(jnp.where(mag <= _NUM_HI, 1.0, 0.0), axis=0, keepdims=True)
        ok = ((den >= _SUM_LO) & (den <= _SUM_HI)
              & (jnp.max(mag[:Dh], axis=0, keepdims=True) >= _NUM_LO))
        return jnp.where(ok, finite, 0.0)

    def step(i, j, p_cur, p_nxt):
        acc = None
        if p_nxt is not None:
            g, q = q_weights(j)
        for c in range(S // _KC):
            ks = slice(c * _KC, (c + 1) * _KC)
            o = _dot(vt_ref[i // nq, :, ks], p_cur[ks, :])
            acc = o if acc is None else acc + o
            if p_nxt is not None:
                p_nxt[ks, :] = jnp.exp2(_dot(k_ref[g, ks, :], q)).astype(_BF)
        store_o(i, acc)
        return in_range(acc)

    def body(n, ok):
        for t in range(_UN):
            j = n * _UN + t
            bufs = (p1_ref, p0_ref) if t % 2 == 0 else (p0_ref, p1_ref)
            ok_t = step(jnp.maximum(j - 1, 0), j, *bufs)
            if t == 0:
                ok_t = jnp.where(n == 0, 1.0, ok_t)
            ok = jnp.minimum(ok, ok_t)
        return ok

    wo_cp.wait()
    ok = jax.lax.fori_loop(0, n_steps // _UN, body, jnp.ones((1, _BQ), _F32))
    wo = wo_ref[...].astype(_F32)
    zrow = jnp.zeros((_HP - Dh, D), _F32)
    wo_pad = jnp.concatenate(
        [t for h in range(_H) for t in (wo[h * Dh:(h + 1) * Dh], zrow)], axis=0)
    wot_ref[...] = wo_pad.T.astype(_BF)

    ok = jnp.minimum(ok, step(n_steps - 1, None, p1_ref, None))

    @pl.when(jnp.min(ok) < 0.5)
    def _():
        def safe_step(i, _):
            g, q = q_weights(i)
            s = _dot(k_ref[g], q)
            p = jnp.exp2(s - jnp.max(s, axis=0, keepdims=True)).astype(_BF)
            store_o(i, _dot(vt_ref[i // nq], p))

        jax.lax.fori_loop(0, n_steps, safe_step, None)

    def out_proj(c):
        sl = _chunk(c, _SC)
        h1 = x_ref[:, sl].astype(_F32) + _dot(wot_ref[...], ot_ref[:, sl])
        ht_ref[:, sl] = h1 + b2_ref[:, sl]
        return _ln_t(h1)

    w1_cp.wait()
    for c in range(S // (2 * _SC)):
        lo, hi = out_proj(c), out_proj(c + S // (2 * _SC))
        _store_lhs(hn_ref, _chunk(c, _SC), lo[:Dm], hi[:Dm], lo[Dm:], hi[Dm:])

    def mlp_up(c, _):
        left, right = _chunk(c, _FC), _chunk(c + F // (2 * _FC), _FC)
        u11, u12, u21, u22 = _strassen(hn_ref, w1_ref, left, right, _ORDER_UP)
        b_l, b_r = b1_ref[:, left], b1_ref[:, right]
        _store_lhs(g_ref, left, _gelu(u11 + b_l), _gelu(u12 + b_r),
                   _gelu(u21 + b_l), _gelu(u22 + b_r))

    def out_copies(c):
        n = S // (2 * _EC)
        return [pltpu.make_async_copy(ob_ref.at[:, _chunk(j, _EC)], out_hbm.at[:, _chunk(j, _EC)],
                                      o_sem.at[j]) for j in (c, c + n)]

    def mlp_down(c, _):
        left, right = _chunk(c, _EC), _chunk(c + S // (2 * _EC), _EC)
        y11, y12, y21, y22 = _strassen(g_ref, w2_ref, left, right, _ORDER_DOWN)
        for rows, cols, y in ((slice(0, Dm), left, y11), (slice(0, Dm), right, y12),
                              (slice(Dm, D), left, y21), (slice(Dm, D), right, y22)):
            ob_ref[rows, cols] = (ht_ref[rows, cols] + y).astype(_BF)
        for cp in out_copies(c):
            cp.start()

    jax.lax.fori_loop(0, F // (2 * _FC), mlp_up, None)
    w2_cp.wait()
    jax.lax.fori_loop(0, S // (2 * _EC), mlp_down, None)
    for c in range(S // (2 * _EC)):
        for cp in out_copies(c):
            cp.wait()


@jax.jit
def pallas_sequential_preLN__mha_block__mixer_token_mlp__prompt_kernel(
    A_x: jax.Array,
    A_wqkv: jax.Array,
    A_wo: jax.Array,
    B_x: jax.Array,
    B_w1: jax.Array,
    B_b1: jax.Array,
    B_w2: jax.Array,
    B_b2: jax.Array,
):
    del B_x
    B, S, D = A_x.shape
    F = B_w1.shape[1]
    assert B == 1
    vmem = pl.BlockSpec(memory_space=pltpu.VMEM)
    hbm = pl.BlockSpec(memory_space=pl.ANY)
    out = pl.pallas_call(
        _kernel,
        out_shape=jax.ShapeDtypeStruct((D, S), A_x.dtype),
        in_specs=[hbm, hbm, hbm, vmem, vmem, hbm, hbm],
        out_specs=hbm,
        scratch_shapes=[
            pltpu.VMEM((D, S), _BF),
            pltpu.VMEM((D, D), _BF),
            pltpu.VMEM((D, 2 * D), _BF),
            pltpu.VMEM((D, D), _BF),
            pltpu.VMEM((S, F), _BF),
            pltpu.VMEM((F, S), _BF),
            pltpu.VMEM((1, F), _F32),
            pltpu.VMEM((1, S), _F32),
            pltpu.VMEM((D, S), _F32),
            pltpu.VMEM((D, S), _F32),
            pltpu.VMEM((_H // _G, S, 128), _BF),
            pltpu.VMEM((_H, _HP, S), _BF),
            pltpu.VMEM((_H * _HP, S), _BF),
            pltpu.VMEM((S, _BQ), _BF),
            pltpu.VMEM((S, _BQ), _BF),
            pltpu.VMEM((7, D // 2, S // 2), _BF),
            pltpu.VMEM((7, D // 2, F // 2), _BF),
            pltpu.VMEM((D, S), _BF),
            pltpu.VMEM((D, _H * _HP), _BF),
            pltpu.SemaphoreType.DMA((7,)),
            pltpu.SemaphoreType.DMA((S // _EC,)),
        ],
        compiler_params=pltpu.CompilerParams(vmem_limit_bytes=100 * 1024 * 1024),
    )(A_x.reshape(S, D).T, A_wqkv, A_wo, B_b1, B_b2, B_w1, B_w2)
    return out.T.reshape(B, S, D)
```
